```python
import jax
import jax.numpy as jnp

def _softmax(x, axis=-1):
    return jax.nn.softmax(x, axis=axis)
def _gelu(x):
    return jax.nn.gelu(x, approximate=True)
def _silu(x):
    return jax.nn.silu(x)
def _sigmoid(x):
    return jax.nn.sigmoid(x)
def _layernorm(x, axis=-1, eps=1e-5):
    m = jnp.mean(x, axis=axis, keepdims=True)
    v = jnp.var(x, axis=axis, keepdims=True)
    return (x - m) / jnp.sqrt(v + eps)
def _scatter_add(tgt, idx, src, axis=0):
    return tgt.at[idx].add(src)
def _segment_sum(src, seg, n):
    return jax.ops.segment_sum(src, seg, n)
class _Rng:
    def __init__(self, key):
        self._k = key
    def _next(self):
        self._k, sub = jax.random.split(self._k)
        return sub
    def normal(self, shape):
        return jax.random.normal(self._next(), shape, dtype=jnp.bfloat16)
    def randint(self, lo, hi, shape):
        return jax.random.randint(self._next(), shape, lo, hi, dtype=jnp.int32)
    def uniform(self, shape, lo=0.0, hi=1.0):
        return jax.random.uniform(self._next(), shape, jnp.bfloat16, lo, hi)
    def permutation(self, n):
        return jax.random.permutation(self._next(), n)


kernel_name = 'recurrent_scan__sliding_local_dilated__swiglu_ffn__prompt'

def setup_inputs():
    _rng = _Rng(jax.random.key(int.from_bytes(__import__("os").urandom(4), "little")))
    _w = (lambda a: (lambda t: t.astype(jnp.bfloat16) if jnp.issubdtype(t.dtype, jnp.floating) else t)(jnp.asarray(a)))
    def _A_setup():
        B, S, D = 1, 2048, 1024
        return {
            "x": _w((lambda *s: _rng.normal(s) * 0.05)(B, S, D)),
            "wqkv": _w((lambda *s: _rng.normal(s) * 0.05)(D, 3 * D)),
            "wo": _w((lambda *s: _rng.normal(s) * 0.05)(D, D)),
        }
    _A_in = _A_setup()

    def _B_setup():
        B, S, D, F = 1, 2048, 1024, 3584
        return {
            "x": _w((lambda *s: _rng.normal(s) * 0.05)(B, S, D)),
            "w_gate": _w((lambda *s: _rng.normal(s) * 0.05)(D, F)),
            "w_up": _w((lambda *s: _rng.normal(s) * 0.05)(D, F)),
            "w_down": _w((lambda *s: _rng.normal(s) * 0.05)(F, D)),
        }
    _B_in = _B_setup()

    return {
        "A_x": _A_in["x"],
        "A_wqkv": _A_in["wqkv"],
        "A_wo": _A_in["wo"],
        "B_x": _B_in["x"],
        "B_w_gate": _B_in["w_gate"],
        "B_w_up": _B_in["w_up"],
        "B_w_down": _B_in["w_down"],
    }

def reference(A_x, A_wqkv, A_wo, B_x, B_w_gate, B_w_up, B_w_down):
    def _A_ref(x, wqkv, wo):
        B, S, D = x.shape
        H = 32; Dh = D // H
        W, dil = 8, 2
        qkv = (lambda x, *d: x.transpose(*d))((x @ wqkv).reshape(B, S, 3, H, Dh), 2, 0, 3, 1, 4)
        q, k, v = qkv[0], qkv[1], qkv[2]
        scale = Dh ** -0.5
        pos = jnp.arange(S)
        off = jnp.arange(W) * dil
        idx = pos[:, None] - off[None, :]
        mask = idx >= 0
        idx_c = jnp.where(mask, idx, 0).reshape(-1)
        kg = k[:, :, idx_c, :].reshape(B, H, S, W, Dh)
        vg = v[:, :, idx_c, :].reshape(B, H, S, W, Dh)
        logits = jnp.einsum("bhsd,bhswd->bhsw", q, kg) * scale
        logits = jnp.where(mask[None, None, :, :], logits, -1e9)
        attn = _softmax(logits, axis=-1)
        o = jnp.einsum("bhsw,bhswd->bhsd", attn, vg)
        return (lambda x, *d: x.transpose(*d))(o, 0, 2, 1, 3).reshape(B, S, D) @ wo

    def _B_ref(x, w_gate, w_up, w_down):
        g = _silu(x @ w_gate)
        u = x @ w_up
        return (g * u) @ w_down

    x = A_x
    xn = _layernorm(x, axis=-1)
    s = _A_ref(xn, A_wqkv, A_wo)
    g = _silu(_B_ref(xn, B_w_gate, B_w_up, B_w_down))
    return x + s * g
```

```python
import functools
import jax
import jax.numpy as jnp
from jax import lax
import jax.experimental.pallas as pl
import jax.experimental.pallas.tpu as pltpu

H = 32
W = 8
DIL = 2
HALO = 16
NT = 8
EPS = 1e-5

F32 = jnp.float32
BF16 = jnp.bfloat16
U32 = jnp.uint32


def _lane_masks(rows):
    lane = lax.broadcasted_iota(jnp.int32, (rows, 128), 1)
    return [((lane >> (2 + k)) & 1) == 1 for k in range(3)]


def _tile_select(T, grp):
    X = [T[(-u) % NT] for u in range(NT)]
    for k in range(3):
        X = [jnp.where(grp[k], X[(t - (1 << k)) % NT], X[t]) for t in range(NT)]
    return X


def _permute_tiles(T, grp):
    A = [pltpu.roll(T[j], 4 * j, 1) if j else T[j] for j in range(NT)]
    X = _tile_select(A, grp)
    return [pltpu.roll(X[t], 128 - 4 * t, 1) if t else X[t] for t in range(NT)]


def _unpermute_tiles(T, grp):
    X = [pltpu.roll(T[t], 4 * t, 1) if t else T[t] for t in range(NT)]
    Y = _tile_select(X, grp)
    return [pltpu.roll(Y[j], 128 - 4 * j, 1) if j else Y[j] for j in range(NT)]


def _silu(x):
    return x * jax.nn.sigmoid(x)


def _dot(a, b):
    return jnp.dot(a, b, preferred_element_type=F32)


def make_kernel(S, D, F, cfg):
    tm = cfg["tm"]
    fc = cfg["fc"]
    pc = cfg["pc"]
    slab = cfg["slab"]
    n_tiles = S // tm
    n_fc = F // fc
    n_pc = F // pc
    scale = (D // H) ** -0.5
    NX = 6
    hrows = D // 2
    n_slabs = tm // slab
    NB = n_pc - NX
    slabs_per_b = -(-n_slabs // NB)

    def kernel(x_hbm, wqkv_hbm, wo_hbm, wg_hbm, wu_hbm, wd_hbm, out_hbm,
               x_s, out_s, wqkv_s, wo_s, wg_s, wu_s, wd_s, xn_s, qkv_s, o_s, acc_s,
               x_sem, out_sem, wqkv_sem, wo_sem, wg_sem, wu_sem, wd_sem):

        def rows_of(i):
            return pl.ds(pl.multiple_of(i * tm, tm), tm) if not isinstance(i, int) else pl.ds(i * tm, tm)

        def x_copy(i):
            return pltpu.make_async_copy(x_hbm.at[rows_of(i), :], x_s.at[rows_of(i), :], x_sem.at[i])

        def out_copy(i):
            return pltpu.make_async_copy(out_s.at[rows_of(i), :], out_hbm.at[rows_of(i), :], out_sem.at[i])

        def cols_of(c, n):
            return pl.ds(pl.multiple_of(c * n, n), n) if not isinstance(c, int) else pl.ds(c * n, n)

        def wg_copy(c):
            return pltpu.make_async_copy(wg_hbm.at[:, cols_of(c, pc)], wg_s.at[:, cols_of(c, pc)], wg_sem.at[c])

        def wu_copy(c):
            return pltpu.make_async_copy(wu_hbm.at[:, cols_of(c, pc)], wu_s.at[:, cols_of(c, pc)], wu_sem.at[c])

        def wd_copy(c):
            return pltpu.make_async_copy(wd_hbm.at[cols_of(c, pc), :], wd_s.at[cols_of(c, pc), :], wd_sem.at[c])

        def wqkv_copy(j):
            if isinstance(j, int):
                m, hh = j // 2, j % 2
            else:
                m, hh = j >> 1, j & 1
            return pltpu.make_async_copy(wqkv_hbm.at[cols_of(hh, hrows), cols_of(m, D)],
                                         wqkv_s.at[m, cols_of(hh, hrows), :], wqkv_sem.at[j])

        def wo_copy():
            return pltpu.make_async_copy(wo_hbm, wo_s, wo_sem)

        def layernorm_to(src_rows, dst):
            x = x_s[src_rows, :].astype(F32)
            mean = jnp.mean(x, axis=-1, keepdims=True)
            xc = x - mean
            var = jnp.mean(xc * xc, axis=-1, keepdims=True)
            dst[...] = (xc * lax.rsqrt(var + EPS)).astype(BF16)

        def ffn_hidden(xn, cols):
            g = _dot(xn, wg_s[:, cols])
            u = _dot(xn, wu_s[:, cols])
            h = (_silu(g) * u).astype(BF16)
            return _dot(h, wd_s[cols, :])

        def permute_rows(m, row0, nrows, step):
            grp = _lane_masks(step // 2)
            view = wqkv_s.at[m, pl.ds(row0, nrows), :]
            for r in range(0, nrows, step):
                T = [pltpu.bitcast(view[r:r + step, j * 128:(j + 1) * 128], U32) for j in range(NT)]
                P = _permute_tiles(T, grp)
                for t in range(NT):
                    view[r:r + step, t * 128:(t + 1) * 128] = pltpu.bitcast(P[t], BF16)

        def attention_slab(r0, masked):
            lane = lax.broadcasted_iota(jnp.int32, (slab, 128), 1)
            b0 = (lane & 1) == 0
            b1 = (lane & 2) == 0
            win = pl.ds(r0, HALO + slab)
            L = [None] * W
            for t in range(NT):
                qt = qkv_s[0, t, pl.ds(r0 + HALO, slab), :]
                kv = qkv_s.at[1, t, win, :]
                for w in range(W):
                    off = HALO - DIL * w
                    p = qt * kv[off:off + slab, :]
                    L[w] = p if L[w] is None else L[w] + p
            Z = []
            if masked:
                row = lax.broadcasted_iota(jnp.int32, (slab, 128), 0) + r0
            for w in range(W):
                a = L[w]
                a = a + jnp.where(b0, pltpu.roll(a, 127, 1), pltpu.roll(a, 1, 1))
                a = a + jnp.where(b1, pltpu.roll(a, 126, 1), pltpu.roll(a, 2, 1))
                z = a * scale
                if masked and w > 0:
                    z = jnp.where(row >= DIL * w, z, -1e9)
                Z.append(z)
            mx = functools.reduce(jnp.maximum, Z)
            E = [jnp.exp(z - mx) for z in Z]
            den = functools.reduce(lambda a, b: a + b, E)
            rinv = 1.0 / den
            P = [e * rinv for e in E]
            O = []
            for t in range(NT):
                vv = qkv_s.at[2, t, win, :]
                acc = None
                for w in range(W):
                    off = HALO - DIL * w
                    p = P[w] * vv[off:off + slab, :]
                    acc = p if acc is None else acc + p
                O.append(pltpu.bitcast(acc.astype(BF16), U32))
            O = _unpermute_tiles(O, _lane_masks(slab // 2))
            for j in range(NT):
                o_s[pl.ds(r0, slab), j * 128:(j + 1) * 128] = pltpu.bitcast(O[j], BF16)

        def carry_halo():
            for m in (1, 2):
                for t in range(NT):
                    qkv_s[m, t, 0:HALO, :] = qkv_s[m, t, tm:tm + HALO, :]

        x_copy(0).start()

        def start_x_phase(c, carry):
            wg_copy(c).start()
            wu_copy(c).start()
            wqkv_copy(c).start()
            wd_copy(c).start()
            return carry
        lax.fori_loop(0, NX, start_x_phase, 0)

        def start_b_phase(c, carry):
            wg_copy(c).start()
            wu_copy(c).start()
            wd_copy(c).start()
            return carry
        lax.fori_loop(NX, n_pc, start_b_phase, 0)
        wo_copy().start()

        def start_x_rest(i, carry):
            x_copy(i).start()
            return carry
        lax.fori_loop(1, n_tiles, start_x_rest, 0)

        zeros_halo = jnp.zeros((HALO, 128), F32)
        for m in (1, 2):
            for t in range(NT):
                qkv_s[m, t, 0:HALO, :] = zeros_halo
        acc_s[...] = jnp.zeros((tm, D), F32)

        x_copy(0).wait()
        lnr = cfg["ln_rows"]

        def ln0_body(j, carry):
            rr = pl.ds(pl.multiple_of(j * lnr, lnr), lnr)
            layernorm_to(rr, xn_s.at[0, rr, :])
            return carry
        lax.fori_loop(0, tm // lnr, ln0_body, 0)

        def x_body(m, carry):
            def half_body(hh, carry2):
                c = 2 * m + hh
                wg_copy(c).wait()
                wu_copy(c).wait()
                wd_copy(c).wait()
                wqkv_copy(c).wait()
                acc_s[...] += ffn_hidden(xn_s[0], cols_of(c, pc))
                permute_rows(m, pl.multiple_of(hh * hrows, hrows), hrows, cfg["prow"])
                return carry2
            lax.fori_loop(0, 2, half_body, 0)

            nq = cfg["nq"]

            def proj_body(nh, carry2):
                r = _dot(xn_s[0], wqkv_s[m, :, cols_of(nh, nq)])
                for tt in range(nq // 128):
                    qkv_s[m, nh * (nq // 128) + tt, HALO:HALO + tm, :] = r[:, tt * 128:(tt + 1) * 128]
                return carry2
            lax.fori_loop(0, D // nq, proj_body, 0)
            return carry
        lax.fori_loop(0, 3, x_body, 0)

        def b_body(j, carry):
            c = NX + j
            wg_copy(c).wait()
            wu_copy(c).wait()
            wd_copy(c).wait()
            acc_s[...] += ffn_hidden(xn_s[0], cols_of(c, pc))
            for s in range(slabs_per_b):
                sl = jnp.minimum(j * slabs_per_b + s, n_slabs - 1)
                attention_slab(pl.multiple_of(sl * slab, slab), True)
            return carry
        lax.fori_loop(0, NB, b_body, 0)
        carry_halo()

        wo_copy().wait()
        x_copy(1).wait()
        tr = cfg["tail_rows"]

        def tail_body(j, carry):
            rr = pl.ds(pl.multiple_of(j * tr, tr), tr)
            s = _dot(o_s[rr, :], wo_s[...])
            res = x_s[rr, :].astype(F32) + s * _silu(acc_s[rr, :])
            out_s[rr, :] = res.astype(BF16)
            r1 = pl.ds(pl.multiple_of(tm + j * tr, tr), tr)
            layernorm_to(r1, xn_s.at[1, rr, :])
            return carry
        lax.fori_loop(0, tm // tr, tail_body, 0)
        out_copy(0).start()

        def tile_body(i, carry):
            slot = i & 1
            nxt = jnp.minimum(i + 1, n_tiles - 1)

            @pl.when(i + 1 < n_tiles)
            def _():
                x_copy(i + 1).wait()

            xn = xn_s[slot]
            for m in range(3):
                r = _dot(xn, wqkv_s[m])
                for t in range(NT):
                    qkv_s[m, t, HALO:HALO + tm, :] = r[:, t * 128:(t + 1) * 128]

            acc = None
            done = 0
            na = cfg["n_att"]
            for c in range(n_fc):
                d = ffn_hidden(xn, pl.ds(c * fc, fc))
                acc = d if acc is None else acc + d
                upto = min(n_slabs, -(-n_slabs * (c + 1) // na))
                for sl in range(done, upto):
                    attention_slab(sl * slab, False)
                done = upto
                if c == cfg["ln_at"]:
                    layernorm_to(rows_of(nxt), xn_s.at[1 - slot])
            carry_halo()

            s = _dot(o_s[...], wo_s[...])
            res = x_s[rows_of(i), :].astype(F32) + s * _silu(acc)
            out_s[rows_of(i), :] = res.astype(BF16)
            out_copy(i).start()
            return carry

        lax.fori_loop(1, n_tiles, tile_body, 0)
        for i in range(n_tiles):
            out_copy(i).wait()

    return kernel


DEFAULT = dict(tm=256, fc=512, pc=256, slab=16, prow=64, ln_rows=64, nq=512, tail_rows=128,
               n_att=4, ln_at=5, vmem_mb=100)


def build(**over):
    cfg = dict(DEFAULT)
    cfg.update(over)

    def fn(A_x, A_wqkv, A_wo, B_x, B_w_gate, B_w_up, B_w_down):
        Bsz, S, D = A_x.shape
        F = B_w_gate.shape[1]
        tm = cfg["tm"]
        n_tiles = S // tm
        n_pc = F // cfg["pc"]
        x2 = A_x.reshape(S, D)
        any_spec = pl.BlockSpec(memory_space=pl.ANY)
        out = pl.pallas_call(
            make_kernel(S, D, F, cfg),
            in_specs=[any_spec] * 6,
            out_specs=any_spec,
            out_shape=jax.ShapeDtypeStruct((S, D), A_x.dtype),
            scratch_shapes=[
                pltpu.VMEM((S, D), BF16),
                pltpu.VMEM((S, D), BF16),
                pltpu.VMEM((3, D, D), BF16),
                pltpu.VMEM((D, D), BF16),
                pltpu.VMEM((D, F), BF16),
                pltpu.VMEM((D, F), BF16),
                pltpu.VMEM((F, D), BF16),
                pltpu.VMEM((2, tm, D), BF16),
                pltpu.VMEM((3, NT, HALO + tm, 128), F32),
                pltpu.VMEM((tm, D), BF16),
                pltpu.VMEM((tm, D), F32),
                pltpu.SemaphoreType.DMA((n_tiles,)),
                pltpu.SemaphoreType.DMA((n_tiles,)),
                pltpu.SemaphoreType.DMA((6,)),
                pltpu.SemaphoreType.DMA(()),
                pltpu.SemaphoreType.DMA((n_pc,)),
                pltpu.SemaphoreType.DMA((n_pc,)),
                pltpu.SemaphoreType.DMA((n_pc,)),
            ],
            compiler_params=pltpu.CompilerParams(vmem_limit_bytes=cfg["vmem_mb"] * 2 ** 20),
            name="fused_block",
        )(x2, A_wqkv, A_wo, B_w_gate, B_w_up, B_w_down)
        return out.reshape(Bsz, S, D)
    return fn


_fn = build()


@jax.jit
def pallas_recurrent_scan__sliding_local_dilated__swiglu_ffn__prompt_kernel(
    A_x: jax.Array,
    A_wqkv: jax.Array,
    A_wo: jax.Array,
    B_x: jax.Array,
    B_w_gate: jax.Array,
    B_w_up: jax.Array,
    B_w_down: jax.Array,
):
    return _fn(A_x, A_wqkv, A_wo, B_x, B_w_gate, B_w_up, B_w_down)
```

```python
import functools
import jax
import jax.numpy as jnp
from jax import lax
import jax.experimental.pallas as pl
import jax.experimental.pallas.tpu as pltpu

H = 32
W = 8
DIL = 2
HALO = 16
NT = 8
EPS = 1e-5

F32 = jnp.float32
BF16 = jnp.bfloat16
U32 = jnp.uint32


def _lane_masks(rows):
    lane = lax.broadcasted_iota(jnp.int32, (rows, 128), 1)
    return [((lane >> (2 + k)) & 1) == 1 for k in range(3)]


def _tile_select(T, grp):
    X = [T[(-u) % NT] for u in range(NT)]
    for k in range(3):
        X = [jnp.where(grp[k], X[(t - (1 << k)) % NT], X[t]) for t in range(NT)]
    return X


def _permute_tiles(T, grp):
    A = [pltpu.roll(T[j], 4 * j, 1) if j else T[j] for j in range(NT)]
    X = _tile_select(A, grp)
    return [pltpu.roll(X[t], 128 - 4 * t, 1) if t else X[t] for t in range(NT)]


def _unpermute_tiles(T, grp):
    X = [pltpu.roll(T[t], 4 * t, 1) if t else T[t] for t in range(NT)]
    Y = _tile_select(X, grp)
    return [pltpu.roll(Y[j], 128 - 4 * j, 1) if j else Y[j] for j in range(NT)]


def _silu(x):
    return x * pl.reciprocal(1.0 + jnp.exp(-x), approx=True)


def _dot(a, b):
    return jnp.dot(a, b, preferred_element_type=F32)


def _ld(words):
    return pltpu.bitcast(words, BF16)


def _pk(rows):
    return pltpu.bitcast(rows, U32)


def make_kernel(S, D, F, cfg):
    tm = cfg["tm"]
    fc = cfg["fc"]
    pc = cfg["pc"]
    slab = cfg["slab"]
    n_tiles = S // tm
    n_fc = F // fc
    n_pc = F // pc
    scale = (D // H) ** -0.5
    NX = 6
    hwords = D // 4
    n_slabs = tm // slab
    NB = n_pc - NX
    slabs_per_b = -(-n_slabs // NB)

    def kernel(x_hbm, wqkv_hbm, wo_hbm, wg_hbm, wu_hbm, wd_hbm, out_hbm,
               x_s, out_s, wqkv_s, wo_s, wg_s, wu_s, wd_s, xn_s, qkv_s, o_s, aq_s,
               x_sem, out_sem, wqkv_sem, wo_sem, wg_sem, wu_sem, wd_sem):

        hm = tm // 2
        x_w, out_w = x_hbm.bitcast(U32), out_hbm.bitcast(U32)
        wqkv_w, wo_w = wqkv_hbm.bitcast(U32), wo_hbm.bitcast(U32)
        wg_w, wu_w, wd_w = wg_hbm.bitcast(U32), wu_hbm.bitcast(U32), wd_hbm.bitcast(U32)

        def span(c, n):
            return pl.ds(pl.multiple_of(c * n, n), n) if not isinstance(c, int) else pl.ds(c * n, n)

        def words_of(i):
            return span(i, hm)

        def x_copy(i):
            return pltpu.make_async_copy(x_w.at[words_of(i), :], x_s.at[words_of(i), :], x_sem.at[i])

        def out_copy(i):
            return pltpu.make_async_copy(out_s.at[words_of(i), :], out_w.at[words_of(i), :], out_sem.at[i])

        def wg_copy(c):
            return pltpu.make_async_copy(wg_w.at[:, span(c, pc)], wg_s.at[:, span(c, pc)], wg_sem.at[c])

        def wu_copy(c):
            return pltpu.make_async_copy(wu_w.at[:, span(c, pc)], wu_s.at[:, span(c, pc)], wu_sem.at[c])

        def wd_copy(c):
            return pltpu.make_async_copy(wd_w.at[span(c, pc // 2), :], wd_s.at[span(c, pc // 2), :], wd_sem.at[c])

        def wqkv_copy(j):
            if isinstance(j, int):
                m, hh = j // 2, j % 2
            else:
                m, hh = j >> 1, j & 1
            return pltpu.make_async_copy(wqkv_w.at[span(hh, hwords), span(m, D)],
                                         wqkv_s.at[m, span(hh, hwords), :], wqkv_sem.at[j])

        def wo_copy():
            return pltpu.make_async_copy(wo_w, wo_s, wo_sem)

        def layernorm_to(src_words, dst):
            x = _ld(x_s[src_words, :]).astype(F32)
            mean = jnp.mean(x, axis=-1, keepdims=True)
            xc = x - mean
            var = jnp.mean(xc * xc, axis=-1, keepdims=True)
            dst[...] = _pk((xc * lax.rsqrt(var + EPS)).astype(BF16))

        def ffn_hidden(xn, c, n):
            g = _dot(xn, _ld(wg_s[:, span(c, n)]))
            u = _dot(xn, _ld(wu_s[:, span(c, n)]))
            h = (_silu(g) * u).astype(BF16)
            return _dot(h, _ld(wd_s[span(c, n // 2), :]))

        def permute_words(m, hh, step):
            grp = _lane_masks(step)
            view = wqkv_s.at[m, span(hh, hwords), :]
            for r in range(0, hwords, step):
                T = [view[r:r + step, j * 128:(j + 1) * 128] for j in range(NT)]
                P = _permute_tiles(T, grp)
                for t in range(NT):
                    view[r:r + step, t * 128:(t + 1) * 128] = P[t]

        def attention_slab(r0, masked, q_get, o_put=None):
            lane = lax.broadcasted_iota(jnp.int32, (slab, 128), 1)
            b0 = (lane & 1) == 0
            b1 = (lane & 2) == 0
            win = pl.ds(r0, HALO + slab)
            L = [None] * W
            for t in range(NT):
                qt = q_get(r0, t)
                kv = qkv_s.at[1, t, win, :]
                for w in range(W):
                    off = HALO - DIL * w
                    p = qt * kv[off:off + slab, :]
                    L[w] = p if L[w] is None else L[w] + p
            Z = []
            if masked:
                row = lax.broadcasted_iota(jnp.int32, (slab, 128), 0) + r0
            for w in range(W):
                a = L[w]
                a = a + jnp.where(b0, pltpu.roll(a, 127, 1), pltpu.roll(a, 1, 1))
                a = a + jnp.where(b1, pltpu.roll(a, 126, 1), pltpu.roll(a, 2, 1))
                z = a * scale
                if masked and w > 0:
                    z = jnp.where(row >= DIL * w, z, -1e9)
                Z.append(z)
            mx = functools.reduce(jnp.maximum, Z)
            E = [jnp.exp(z - mx) for z in Z]
            den = functools.reduce(lambda a, b: a + b, E)
            rinv = pl.reciprocal(den, approx=True)
            P = [e * rinv for e in E]
            O = []
            for t in range(NT):
                vv = qkv_s.at[2, t, win, :]
                acc = None
                for w in range(W):
                    off = HALO - DIL * w
                    p = P[w] * vv[off:off + slab, :]
                    acc = p if acc is None else acc + p
                O.append(_pk(acc.astype(BF16)))
            O = _unpermute_tiles(O, _lane_masks(slab // 2))
            for j in range(NT):
                o_put(r0, j, O[j])

        def put_o_scratch(r0, j, val):
            if isinstance(r0, int):
                o_s[r0 // 2:(r0 + slab) // 2, j * 128:(j + 1) * 128] = val
            else:
                o_s[pl.ds(pl.multiple_of(r0 >> 1, slab // 2), slab // 2), j * 128:(j + 1) * 128] = val

        def carry_halo():
            for m in (1, 2):
                for t in range(NT):
                    qkv_s[m, t, 0:HALO, :] = qkv_s[m, t, tm:tm + HALO, :]

        x_copy(0).start()

        def start_x_phase(c, carry):
            wg_copy(c).start()
            wu_copy(c).start()
            wqkv_copy(c).start()
            wd_copy(c).start()
            return carry
        lax.fori_loop(0, NX, start_x_phase, 0)

        def start_b_phase(c, carry):
            wg_copy(c).start()
            wu_copy(c).start()
            wd_copy(c).start()
            return carry
        lax.fori_loop(NX, n_pc, start_b_phase, 0)
        wo_copy().start()

        def start_x_rest(i, carry):
            x_copy(i).start()
            return carry
        lax.fori_loop(1, n_tiles, start_x_rest, 0)

        zeros_halo = jnp.zeros((HALO, 128), F32)
        for m in (1, 2):
            for t in range(NT):
                qkv_s[m, t, 0:HALO, :] = zeros_halo
        aq_s[0] = jnp.zeros((tm, D), F32)

        x_copy(0).wait()
        lnr = cfg["ln_rows"]

        def ln0_body(j, carry):
            rr = span(j, lnr // 2)
            layernorm_to(rr, xn_s.at[0, rr, :])
            return carry
        lax.fori_loop(0, tm // lnr, ln0_body, 0)

        def x_body(m, carry):
            def half_body(hh, carry2):
                c = 2 * m + hh
                wg_copy(c).wait()
                wu_copy(c).wait()
                wd_copy(c).wait()
                wqkv_copy(c).wait()
                aq_s[0] += ffn_hidden(_ld(xn_s[0]), c, pc)
                permute_words(m, hh, cfg["prow"] // 2)
                return carry2
            lax.fori_loop(0, 2, half_body, 0)

            nq = cfg["nq"]

            def proj_body(nh, carry2):
                r = _dot(_ld(xn_s[0]), _ld(wqkv_s[m, :, span(nh, nq)]))
                for tt in range(nq // 128):
                    qkv_s[m, nh * (nq // 128) + tt, HALO:HALO + tm, :] = r[:, tt * 128:(tt + 1) * 128]
                return carry2
            lax.fori_loop(0, D // nq, proj_body, 0)
            return carry
        lax.fori_loop(0, 3, x_body, 0)

        def b_body(j, carry):
            c = NX + j
            wg_copy(c).wait()
            wu_copy(c).wait()
            wd_copy(c).wait()
            aq_s[0] += ffn_hidden(_ld(xn_s[0]), c, pc)
            for s in range(slabs_per_b):
                sl = jnp.minimum(j * slabs_per_b + s, n_slabs - 1)
                attention_slab(pl.multiple_of(sl * slab, slab), True,
                               lambda r0, t: qkv_s[0, t, pl.ds(r0 + HALO, slab), :], put_o_scratch)
            return carry
        lax.fori_loop(0, NB, b_body, 0)
        carry_halo()

        wo_copy().wait()
        x_copy(1).wait()
        tr = cfg["tail_rows"]

        def tail_body(j, carry):
            rr = span(j, tr)
            rw = span(j, tr // 2)
            s = _dot(_ld(o_s[rw, :]), _ld(wo_s[...]))
            res = _ld(x_s[rw, :]).astype(F32) + s * _silu(aq_s[0, rr, :])
            out_s[rw, :] = _pk(res.astype(BF16))
            layernorm_to(span(j + tm // tr, tr // 2), xn_s.at[1, rw, :])
            return carry
        lax.fori_loop(0, tm // tr, tail_body, 0)
        out_copy(0).start()

        def tile_body(i, carry):
            slot = i & 1
            nxt = jnp.minimum(i + 1, n_tiles - 1)

            @pl.when(i + 1 < n_tiles)
            def _():
                x_copy(i + 1).wait()

            reread = cfg["reread"]
            xn0 = _ld(xn_s[slot])
            get_xn = (lambda: _ld(xn_s[slot])) if reread else (lambda: xn0)
            if cfg["ln_at"] == -2:
                layernorm_to(words_of(nxt), xn_s.at[1 - slot])

            pace = cfg["pace"]
            one = jnp.minimum(i, 1)

            def proj(m):
                r = _dot(get_xn() if reread > 1 else xn0, _ld(wqkv_s[m]))
                if m == 0 and pace:
                    aq_s[one] = r
                else:
                    for t in range(NT):
                        qkv_s[m, t, HALO:HALO + tm, :] = r[:, t * 128:(t + 1) * 128]

            if pace:
                q_get = lambda r0, t: aq_s[one, pl.ds(r0, slab), t * 128:(t + 1) * 128]
            else:
                q_get = lambda r0, t: qkv_s[0, t, pl.ds(r0 + HALO, slab), :]

            two = jnp.minimum(i + 1, 2)
            chain = cfg["chain"]
            if chain:
                def o_put(r0, j, val):
                    aq_s[two, pl.ds(r0 // 2, slab // 2), j * 128:(j + 1) * 128] = pltpu.bitcast(val, F32)
            else:
                o_put = put_o_scratch
            v_at = cfg["v_at"]
            proj(0)
            proj(1)
            if v_at == 0:
                proj(2)
            if cfg["ln_at"] == -1:
                layernorm_to(words_of(nxt), xn_s.at[1 - slot])
            acc = None
            done = 0
            groups = cfg["groups"]
            for c in range(n_fc):
                d = ffn_hidden(get_xn(), c, fc)
                if pace == 1:
                    if c == 0:
                        aq_s[0] = d
                    else:
                        aq_s[0] += d
                else:
                    acc = d if acc is None else acc + d
                if v_at == c + 1:
                    proj(2)
                if c == min(cfg["ln_at"], n_fc - 1):
                    layernorm_to(words_of(nxt), xn_s.at[1 - slot])
                upto = groups[c] if c < len(groups) else n_slabs
                for sl in range(done, min(upto, n_slabs)):
                    attention_slab(sl * slab, False, q_get, o_put)
                done = max(done, min(upto, n_slabs))
            for sl in range(done, n_slabs):
                attention_slab(sl * slab, False, q_get, o_put)
            if pace == 1:
                acc = aq_s[0]
            carry_halo()

            if chain:
                s = _dot(pltpu.bitcast(aq_s[two, 0:tm // 2, :], BF16), _ld(wo_s[...]))
            else:
                s = _dot(_ld(o_s[...]), _ld(wo_s[...]))
            res = _ld(x_s[words_of(i), :]).astype(F32) + s * _silu(acc)
            out_s[words_of(i), :] = _pk(res.astype(BF16))
            out_copy(i).start()
            return carry

        lax.fori_loop(1, n_tiles, tile_body, 0)
        for i in range(n_tiles):
            out_copy(i).wait()

    return kernel


DEFAULT = dict(tm=256, fc=512, pc=256, slab=16, prow=64, ln_rows=64, nq=512, tail_rows=128,
               ln_at=-1, reread=1, v_at=0, chain=0, pace=0, groups=(0, 0, 0, 0, 0, 0, 16), vmem_mb=100, flags=None, name="fused_block")


def build(**over):
    cfg = dict(DEFAULT)
    cfg.update(over)

    def fn(A_x, A_wqkv, A_wo, B_x, B_w_gate, B_w_up, B_w_down):
        Bsz, S, D = A_x.shape
        F = B_w_gate.shape[1]
        tm = cfg["tm"]
        n_tiles = S // tm
        n_pc = F // cfg["pc"]
        x2 = A_x.reshape(S, D)
        any_spec = pl.BlockSpec(memory_space=pl.ANY)
        out = pl.pallas_call(
            make_kernel(S, D, F, cfg),
            in_specs=[any_spec] * 6,
            out_specs=any_spec,
            out_shape=jax.ShapeDtypeStruct((S, D), A_x.dtype),
            scratch_shapes=[
                pltpu.VMEM((S // 2, D), U32),
                pltpu.VMEM((S // 2, D), U32),
                pltpu.VMEM((3, D // 2, D), U32),
                pltpu.VMEM((D // 2, D), U32),
                pltpu.VMEM((D // 2, F), U32),
                pltpu.VMEM((D // 2, F), U32),
                pltpu.VMEM((F // 2, D), U32),
                pltpu.VMEM((2, tm // 2, D), U32),
                pltpu.VMEM((3, NT, HALO + tm, 128), F32),
                pltpu.VMEM((tm // 2, D), U32),
                pltpu.VMEM((3, tm, D), F32),
                pltpu.SemaphoreType.DMA((n_tiles,)),
                pltpu.SemaphoreType.DMA((n_tiles,)),
                pltpu.SemaphoreType.DMA((6,)),
                pltpu.SemaphoreType.DMA(()),
                pltpu.SemaphoreType.DMA((n_pc,)),
                pltpu.SemaphoreType.DMA((n_pc,)),
                pltpu.SemaphoreType.DMA((n_pc,)),
            ],
            compiler_params=pltpu.CompilerParams(vmem_limit_bytes=cfg["vmem_mb"] * 2 ** 20,
                                                 flags=(cfg["flags"] or None)),
            name=cfg["name"],
        )(x2, A_wqkv, A_wo, B_w_gate, B_w_up, B_w_down)
        return out.reshape(Bsz, S, D)
    return fn


_fn = build(groups=(3,6,9,12,16))


@jax.jit
def pallas_recurrent_scan__sliding_local_dilated__swiglu_ffn__prompt_kernel(
    A_x: jax.Array,
    A_wqkv: jax.Array,
    A_wo: jax.Array,
    B_x: jax.Array,
    B_w_gate: jax.Array,
    B_w_up: jax.Array,
    B_w_down: jax.Array,
):
    return _fn(A_x, A_wqkv, A_wo, B_x, B_w_gate, B_w_up, B_w_down)
```

```python
import functools

import jax
import jax.numpy as jnp
from jax import lax
import jax.experimental.pallas as pl
import jax.experimental.pallas.tpu as pltpu

H = 32
W = 8
DIL = 2
HALO = 16
NT = 8
EPS = 1e-5
LOG2E = 1.4426950408889634
MASKED = -1e9

TM = 256
FC = 512
PC = 256
SLAB = 16
PERM_WORDS = 32
LN0_ROWS = 64
PROJ_COLS = 512
TAIL_ROWS = 128
SLABS_AFTER = (3, 6, 9, 12, 16, 16, 16)

F32 = jnp.float32
BF16 = jnp.bfloat16
U32 = jnp.uint32


def _dot(a, b):
    return jnp.dot(a, b, preferred_element_type=F32)


def _ld(words):
    return pltpu.bitcast(words, BF16)


def _pk(rows):
    return pltpu.bitcast(rows, U32)


def _silu(x):
    return x * pl.reciprocal(1.0 + jnp.exp(-x), approx=True)


def _span(i, n):
    return pl.ds(i * n, n) if isinstance(i, int) else pl.ds(pl.multiple_of(i * n, n), n)


def _group_bits(rows):
    lane = lax.broadcasted_iota(jnp.int32, (rows, 128), 1)
    return [((lane >> (2 + k)) & 1) == 1 for k in range(3)]


def _rotate_tiles(tiles, bits):
    x = [tiles[(-u) % NT] for u in range(NT)]
    for k in range(3):
        x = [jnp.where(bits[k], x[(t - (1 << k)) % NT], x[t]) for t in range(NT)]
    return x


def _permute_tiles(tiles, bits):
    x = [pltpu.roll(tiles[j], 4 * j, 1) if j else tiles[j] for j in range(NT)]
    x = _rotate_tiles(x, bits)
    return [pltpu.roll(x[t], 128 - 4 * t, 1) if t else x[t] for t in range(NT)]


def _unpermute_tiles(tiles, bits):
    x = [pltpu.roll(tiles[t], 4 * t, 1) if t else tiles[t] for t in range(NT)]
    x = _rotate_tiles(x, bits)
    return [pltpu.roll(x[j], 128 - 4 * j, 1) if j else x[j] for j in range(NT)]


def _make_kernel(S, D, F):
    n_tiles = S // TM
    n_fc = F // FC
    n_pc = F // PC
    n_slabs = TM // SLAB
    hm = TM // 2
    half = D // 4
    n_x = 6
    n_b = n_pc - n_x
    slabs_per_b = n_slabs // n_b
    assert n_b * slabs_per_b == n_slabs and len(SLABS_AFTER) == n_fc and SLABS_AFTER[-1] == n_slabs
    scale = (D // H) ** -0.5

    def kernel(x_hbm, wqkv_hbm, wo_hbm, wg_hbm, wu_hbm, wd_hbm, out_hbm,
               x_s, out_s, wqkv_s, wo_s, wg_s, wu_s, wd_s, xn_s, qkv_s, o_s, acc_s,
               x_sem, out_sem, w_sem):
        x_w, out_w = x_hbm.bitcast(U32), out_hbm.bitcast(U32)
        wqkv_w, wo_w = wqkv_hbm.bitcast(U32), wo_hbm.bitcast(U32)
        wg_w, wu_w, wd_w = wg_hbm.bitcast(U32), wu_hbm.bitcast(U32), wd_hbm.bitcast(U32)

        def x_copy(i):
            sem = w_sem.at[n_pc] if isinstance(i, int) and i == 1 else x_sem.at[i]
            return pltpu.make_async_copy(x_w.at[_span(i, hm), :], x_s.at[_span(i, hm), :], sem)

        def out_copy(i):
            return pltpu.make_async_copy(out_s.at[_span(i, hm), :], out_w.at[_span(i, hm), :], out_sem)

        def step_copies(c, with_wqkv):
            copies = [
                pltpu.make_async_copy(wg_w.at[:, _span(c, PC)], wg_s.at[:, _span(c, PC)], w_sem.at[c]),
                pltpu.make_async_copy(wu_w.at[:, _span(c, PC)], wu_s.at[:, _span(c, PC)], w_sem.at[c]),
            ]
            if with_wqkv:
                m, hh = c >> 1, c & 1
                copies.append(pltpu.make_async_copy(wqkv_w.at[_span(hh, half), _span(m, D)],
                                                    wqkv_s.at[m, _span(hh, half), :], w_sem.at[c]))
            copies.append(pltpu.make_async_copy(wd_w.at[_span(c, PC // 2), :], wd_s.at[_span(c, PC // 2), :],
                                                w_sem.at[c]))
            return copies

        wo_copy = pltpu.make_async_copy(wo_w, wo_s, w_sem.at[n_pc])

        def layernorm_to(src_words, dst):
            x = _ld(x_s[src_words, :]).astype(F32)
            mean = jnp.mean(x, axis=-1, keepdims=True)
            xc = x - mean
            var = jnp.mean(xc * xc, axis=-1, keepdims=True)
            dst[...] = _pk((xc * lax.rsqrt(var + EPS)).astype(BF16))

        def ffn_step(xn, c, n):
            g = _dot(xn, _ld(wg_s[:, _span(c, n)]))
            u = _dot(xn, _ld(wu_s[:, _span(c, n)]))
            h = (_silu(g) * u).astype(BF16)
            return _dot(h, _ld(wd_s[_span(c, n // 2), :]))

        def permute_half(m, hh):
            bits = _group_bits(PERM_WORDS)
            view = wqkv_s.at[m, _span(hh, half), :]
            for r in range(0, half, PERM_WORDS):
                tiles = [view[r:r + PERM_WORDS, j * 128:(j + 1) * 128] for j in range(NT)]
                for t, val in enumerate(_permute_tiles(tiles, bits)):
                    view[r:r + PERM_WORDS, t * 128:(t + 1) * 128] = val

        def attention_slab(r0, first_tile):
            lane = lax.broadcasted_iota(jnp.int32, (SLAB, 128), 1)
            low1 = (lane & 1) == 0
            low2 = (lane & 2) == 0
            window = pl.ds(r0, HALO + SLAB)
            logit = [None] * W
            for t in range(NT):
                q = qkv_s[0, t, pl.ds(r0 + HALO, SLAB), :]
                k_win = qkv_s.at[1, t, window, :]
                for w in range(W):
                    off = HALO - DIL * w
                    prod = q * k_win[off:off + SLAB, :]
                    logit[w] = prod if logit[w] is None else logit[w] + prod
            if first_tile:
                row = lax.broadcasted_iota(jnp.int32, (SLAB, 128), 0) + r0
            for w in range(W):
                z = logit[w]
                z = z + jnp.where(low1, pltpu.roll(z, 127, 1), pltpu.roll(z, 1, 1))
                z = z + jnp.where(low2, pltpu.roll(z, 126, 1), pltpu.roll(z, 2, 1))
                if first_tile and w > 0:
                    z = jnp.where(row >= DIL * w, z, MASKED / scale)
                logit[w] = z
            top = functools.reduce(jnp.maximum, logit)
            e = [jnp.exp2((z - top) * (scale * LOG2E)) for z in logit]
            rinv = pl.reciprocal(functools.reduce(lambda a, b: a + b, e), approx=True)
            out = []
            for t in range(NT):
                v_win = qkv_s.at[2, t, window, :]
                acc = None
                for w in range(W):
                    off = HALO - DIL * w
                    prod = e[w] * v_win[off:off + SLAB, :]
                    acc = prod if acc is None else acc + prod
                out.append(_pk((acc * rinv).astype(BF16)))
            out = _unpermute_tiles(out, _group_bits(SLAB // 2))
            if isinstance(r0, int):
                words = pl.ds(r0 // 2, SLAB // 2)
            else:
                words = pl.ds(pl.multiple_of(r0 >> 1, SLAB // 2), SLAB // 2)
            for j in range(NT):
                o_s[words, j * 128:(j + 1) * 128] = out[j]

        def carry_halo():
            for m in (1, 2):
                for t in range(NT):
                    qkv_s[m, t, 0:HALO, :] = qkv_s[m, t, TM:TM + HALO, :]

        x_copy(0).start()

        def start_x_step(c, carry):
            for cp in step_copies(c, True):
                cp.start()
            return carry
        lax.fori_loop(0, n_x, start_x_step, 0)

        def start_b_step(c, carry):
            for cp in step_copies(c, False):
                cp.start()
            return carry
        lax.fori_loop(n_x, n_pc, start_b_step, 0)
        wo_copy.start()
        x_copy(1).start()

        def start_x_tile(i, carry):
            x_copy(i).start()
            return carry
        lax.fori_loop(2, n_tiles, start_x_tile, 0)

        for m in (1, 2):
            for t in range(NT):
                qkv_s[m, t, 0:HALO, :] = jnp.zeros((HALO, 128), F32)
        acc_s[...] = jnp.zeros((TM, D), F32)

        x_copy(0).wait()

        def ln0_step(j, carry):
            words = _span(j, LN0_ROWS // 2)
            layernorm_to(words, xn_s.at[0, words, :])
            return carry
        lax.fori_loop(0, TM // LN0_ROWS, ln0_step, 0)

        def x_phase(m, carry):
            def ffn_and_permute(hh, carry2):
                c = 2 * m + hh
                for cp in step_copies(c, True):
                    cp.wait()
                acc_s[...] += ffn_step(_ld(xn_s[0]), c, PC)
                permute_half(m, hh)
                return carry2
            lax.fori_loop(0, 2, ffn_and_permute, 0)

            def project(n, carry2):
                r = _dot(_ld(xn_s[0]), _ld(wqkv_s[m, :, _span(n, PROJ_COLS)]))
                for tt in range(PROJ_COLS // 128):
                    qkv_s[m, n * (PROJ_COLS // 128) + tt, HALO:HALO + TM, :] = r[:, tt * 128:(tt + 1) * 128]
                return carry2
            lax.fori_loop(0, D // PROJ_COLS, project, 0)
            return carry
        lax.fori_loop(0, 3, x_phase, 0)

        def ffn_and_attend(j, carry):
            c = n_x + j
            for cp in step_copies(c, False):
                cp.wait()
            acc_s[...] += ffn_step(_ld(xn_s[0]), c, PC)
            for s in range(slabs_per_b):
                attention_slab(pl.multiple_of((j * slabs_per_b + s) * SLAB, SLAB), True)
            return carry
        lax.fori_loop(0, n_b, ffn_and_attend, 0)
        carry_halo()

        wo_copy.wait()
        x_copy(1).wait()

        def finish_tile0(j, carry):
            rows, words = _span(j, TAIL_ROWS), _span(j, TAIL_ROWS // 2)
            s = _dot(_ld(o_s[words, :]), _ld(wo_s[...]))
            res = _ld(x_s[words, :]).astype(F32) + s * _silu(acc_s[rows, :])
            out_s[words, :] = _pk(res.astype(BF16))
            layernorm_to(_span(j + TM // TAIL_ROWS, TAIL_ROWS // 2), xn_s.at[1, words, :])
            return carry
        lax.fori_loop(0, TM // TAIL_ROWS, finish_tile0, 0)
        out_copy(0).start()

        def tile_body(i, carry):
            slot = i & 1
            nxt = jnp.minimum(i + 1, n_tiles - 1)

            @pl.when(i + 1 < n_tiles)
            def _():
                x_copy(i + 1).wait()

            xn = _ld(xn_s[slot])
            for m in range(3):
                r = _dot(xn, _ld(wqkv_s[m]))
                for t in range(NT):
                    qkv_s[m, t, HALO:HALO + TM, :] = r[:, t * 128:(t + 1) * 128]

            layernorm_to(pl.ds(pl.multiple_of(nxt * hm, hm), hm), xn_s.at[1 - slot])

            acc = None
            done = 0
            for c in range(n_fc):
                d = ffn_step(_ld(xn_s[slot]), c, FC)
                acc = d if acc is None else acc + d
                for sl in range(done, SLABS_AFTER[c]):
                    attention_slab(sl * SLAB, False)
                done = SLABS_AFTER[c]
            carry_halo()

            s = _dot(_ld(o_s[...]), _ld(wo_s[...]))
            res = _ld(x_s[_span(i, hm), :]).astype(F32) + s * _silu(acc)
            out_s[_span(i, hm), :] = _pk(res.astype(BF16))
            out_copy(i).start()
            return carry

        lax.fori_loop(1, n_tiles, tile_body, 0)
        pltpu.make_async_copy(out_s, out_w, out_sem).wait()

    return kernel


def build(name="fused_block"):
    def fn(A_x, A_wqkv, A_wo, B_x, B_w_gate, B_w_up, B_w_down):
        del B_x
        B, S, D = A_x.shape
        F = B_w_gate.shape[1]
        assert B == 1 and D == NT * 128 and S % TM == 0 and S // TM >= 2 and F % FC == 0
        any_spec = pl.BlockSpec(memory_space=pl.ANY)
        out = pl.pallas_call(
            _make_kernel(S, D, F),
            in_specs=[any_spec] * 6,
            out_specs=any_spec,
            out_shape=jax.ShapeDtypeStruct((S, D), A_x.dtype),
            scratch_shapes=[
                pltpu.VMEM((S // 2, D), U32),
                pltpu.VMEM((S // 2, D), U32),
                pltpu.VMEM((3, D // 2, D), U32),
                pltpu.VMEM((D // 2, D), U32),
                pltpu.VMEM((D // 2, F), U32),
                pltpu.VMEM((D // 2, F), U32),
                pltpu.VMEM((F // 2, D), U32),
                pltpu.VMEM((2, TM // 2, D), U32),
                pltpu.VMEM((3, NT, HALO + TM, 128), F32),
                pltpu.VMEM((TM // 2, D), U32),
                pltpu.VMEM((TM, D), F32),
                pltpu.SemaphoreType.DMA((S // TM,)),
                pltpu.SemaphoreType.DMA(()),
                pltpu.SemaphoreType.DMA((F // PC + 1,)),
            ],
            compiler_params=pltpu.CompilerParams(vmem_limit_bytes=100 * 2 ** 20),
            name=name,
        )(A_x.reshape(S, D), A_wqkv, A_wo, B_w_gate, B_w_up, B_w_down)
        return out.reshape(B, S, D)
    return fn


_fused = build()


@jax.jit
def pallas_recurrent_scan__sliding_local_dilated__swiglu_ffn__prompt_kernel(
    A_x: jax.Array,
    A_wqkv: jax.Array,
    A_wo: jax.Array,
    B_x: jax.Array,
    B_w_gate: jax.Array,
    B_w_up: jax.Array,
    B_w_down: jax.Array,
):
    return _fused(A_x, A_wqkv, A_wo, B_x, B_w_gate, B_w_up, B_w_down)
```

```python
import functools

import jax
import jax.numpy as jnp
from jax import lax
import jax.experimental.pallas as pl
import jax.experimental.pallas.tpu as pltpu

H = 32
W = 8
DIL = 2
HALO = 16
NT = 8
EPS = 1e-5
LOG2E = 1.4426950408889634
MASKED = -1e9

TM = 256
FC = 512
PCX = 128
PCB = 256
KPARTS = 4
SLAB = 16
PERM_WORDS = 32
LN0_ROWS = 64
TAIL_ROWS = 128
SLABS_AFTER = (3, 6, 9, 12, 16, 16, 16)

F32 = jnp.float32
BF16 = jnp.bfloat16
U32 = jnp.uint32


def _dot(a, b):
    return jnp.dot(a, b, preferred_element_type=F32)


def _ld(words):
    return pltpu.bitcast(words, BF16)


def _pk(rows):
    return pltpu.bitcast(rows, U32)


def _silu(x):
    return x * pl.reciprocal(1.0 + jnp.exp(-x), approx=True)


def _span(i, n):
    return pl.ds(i * n, n) if isinstance(i, int) else pl.ds(pl.multiple_of(i * n, n), n)


def _group_bits(rows):
    lane = lax.broadcasted_iota(jnp.int32, (rows, 128), 1)
    return [((lane >> (2 + k)) & 1) == 1 for k in range(3)]


def _rotate_tiles(tiles, bits):
    x = [tiles[(-u) % NT] for u in range(NT)]
    for k in range(3):
        x = [jnp.where(bits[k], x[(t - (1 << k)) % NT], x[t]) for t in range(NT)]
    return x


def _permute_tiles(tiles, bits):
    x = [pltpu.roll(tiles[j], 4 * j, 1) if j else tiles[j] for j in range(NT)]
    x = _rotate_tiles(x, bits)
    return [pltpu.roll(x[t], 128 - 4 * t, 1) if t else x[t] for t in range(NT)]


def _unpermute_tiles(tiles, bits):
    x = [pltpu.roll(tiles[t], 4 * t, 1) if t else tiles[t] for t in range(NT)]
    x = _rotate_tiles(x, bits)
    return [pltpu.roll(x[j], 128 - 4 * j, 1) if j else x[j] for j in range(NT)]


def _make_kernel(S, D, F):
    n_tiles = S // TM
    n_fc = F // FC
    n_slabs = TM // SLAB
    hm = TM // 2
    kw = D // 2 // KPARTS
    n_x = 3 * KPARTS
    n_b = (F - n_x * PCX) // PCB
    slabs_per_b = n_slabs // n_b
    assert n_x * PCX + n_b * PCB == F
    assert n_b * slabs_per_b == n_slabs and len(SLABS_AFTER) == n_fc and SLABS_AFTER[-1] == n_slabs
    scale = (D // H) ** -0.5

    def kernel(x_hbm, wqkv_hbm, wo_hbm, wg_hbm, wu_hbm, wd_hbm, out_hbm,
               x_s, out_s, wqkv_s, wo_s, wg_s, wu_s, wd_s, xn_s, qkv_s, o_s, acc_s,
               x_sem, out_sem, w_sem):
        x_w, out_w = x_hbm.bitcast(U32), out_hbm.bitcast(U32)
        wqkv_w, wo_w = wqkv_hbm.bitcast(U32), wo_hbm.bitcast(U32)
        wg_w, wu_w, wd_w = wg_hbm.bitcast(U32), wu_hbm.bitcast(U32), wd_hbm.bitcast(U32)

        def x_copy(i):
            sem = w_sem.at[n_x + n_b] if isinstance(i, int) and i == 1 else x_sem.at[i]
            return pltpu.make_async_copy(x_w.at[_span(i, hm), :], x_s.at[_span(i, hm), :], sem)

        def out_copy(i):
            return pltpu.make_async_copy(out_s.at[_span(i, hm), :], out_w.at[_span(i, hm), :], out_sem)

        def ffn_cols(c, first_phase):
            if first_phase:
                return _span(c, PCX), _span(c, PCX // 2)
            start = n_x * PCX + (c - n_x) * PCB
            return pl.ds(pl.multiple_of(start, PCX), PCB), pl.ds(pl.multiple_of(start >> 1, PCX // 2), PCB // 2)

        def step_copies(c, first_phase):
            cols, drows = ffn_cols(c, first_phase)
            copies = [
                pltpu.make_async_copy(wg_w.at[:, cols], wg_s.at[:, cols], w_sem.at[c]),
                pltpu.make_async_copy(wu_w.at[:, cols], wu_s.at[:, cols], w_sem.at[c]),
            ]
            if first_phase:
                m, part = c // KPARTS, c % KPARTS
                copies.append(pltpu.make_async_copy(wqkv_w.at[_span(part, kw), _span(m, D)],
                                                    wqkv_s.at[m, _span(part, kw), :], w_sem.at[c]))
            copies.append(pltpu.make_async_copy(wd_w.at[drows, :], wd_s.at[drows, :], w_sem.at[c]))
            return copies

        wo_copy = pltpu.make_async_copy(wo_w, wo_s, w_sem.at[n_x + n_b])

        def layernorm_to(src_words, dst):
            x = _ld(x_s[src_words, :]).astype(F32)
            mean = jnp.mean(x, axis=-1, keepdims=True)
            xc = x - mean
            var = jnp.mean(xc * xc, axis=-1, keepdims=True)
            dst[...] = _pk((xc * lax.rsqrt(var + EPS)).astype(BF16))

        def ffn_step(xn, cols, drows):
            g = _dot(xn, _ld(wg_s[:, cols]))
            u = _dot(xn, _ld(wu_s[:, cols]))
            h = (_silu(g) * u).astype(BF16)
            return _dot(h, _ld(wd_s[drows, :]))

        def permute_part(m, part):
            bits = _group_bits(PERM_WORDS)
            view = wqkv_s.at[m, _span(part, kw), :]
            for r in range(0, kw, PERM_WORDS):
                tiles = [view[r:r + PERM_WORDS, j * 128:(j + 1) * 128] for j in range(NT)]
                for t, val in enumerate(_permute_tiles(tiles, bits)):
                    view[r:r + PERM_WORDS, t * 128:(t + 1) * 128] = val

        def attention_slab(r0, first_tile):
            lane = lax.broadcasted_iota(jnp.int32, (SLAB, 128), 1)
            low1 = (lane & 1) == 0
            low2 = (lane & 2) == 0
            window = pl.ds(r0, HALO + SLAB)
            logit = [None] * W
            for t in range(NT):
                q = qkv_s[0, t, pl.ds(r0 + HALO, SLAB), :]
                k_win = qkv_s.at[1, t, window, :]
                for w in range(W):
                    off = HALO - DIL * w
                    prod = q * k_win[off:off + SLAB, :]
                    logit[w] = prod if logit[w] is None else logit[w] + prod
            if first_tile:
                row = lax.broadcasted_iota(jnp.int32, (SLAB, 128), 0) + r0
            for w in range(W):
                z = logit[w]
                z = z + jnp.where(low1, pltpu.roll(z, 127, 1), pltpu.roll(z, 1, 1))
                z = z + jnp.where(low2, pltpu.roll(z, 126, 1), pltpu.roll(z, 2, 1))
                if first_tile and w > 0:
                    z = jnp.where(row >= DIL * w, z, MASKED / scale)
                logit[w] = z
            top = functools.reduce(jnp.maximum, logit)
            e = [jnp.exp2((z - top) * (scale * LOG2E)) for z in logit]
            rinv = pl.reciprocal(functools.reduce(lambda a, b: a + b, e), approx=True)
            out = []
            for t in range(NT):
                v_win = qkv_s.at[2, t, window, :]
                acc = None
                for w in (0, 4, 1, 5, 2, 6, 3, 7):
                    off = HALO - DIL * w
                    prod = e[w] * v_win[off:off + SLAB, :]
                    acc = prod if acc is None else acc + prod
                out.append(_pk((acc * rinv).astype(BF16)))
            out = _unpermute_tiles(out, _group_bits(SLAB // 2))
            if isinstance(r0, int):
                words = pl.ds(r0 // 2, SLAB // 2)
            else:
                words = pl.ds(pl.multiple_of(r0 >> 1, SLAB // 2), SLAB // 2)
            for j in range(NT):
                o_s[words, j * 128:(j + 1) * 128] = out[j]

        def carry_halo():
            for m in (1, 2):
                for t in range(NT):
                    qkv_s[m, t, 0:HALO, :] = qkv_s[m, t, TM:TM + HALO, :]

        x_copy(0).start()

        def start_first_phase(c, carry):
            for cp in step_copies(c, True):
                cp.start()
            return carry
        lax.fori_loop(0, n_x, start_first_phase, 0)

        def start_second_phase(c, carry):
            for cp in step_copies(c, False):
                cp.start()
            return carry
        lax.fori_loop(n_x, n_x + n_b, start_second_phase, 0)

        for m in (1, 2):
            for t in range(NT):
                qkv_s[m, t, 0:HALO, :] = jnp.zeros((HALO, 128), F32)
        for m in range(3):
            for t in range(NT):
                qkv_s[m, t, HALO:HALO + TM, :] = jnp.zeros((TM, 128), F32)
        acc_s[...] = jnp.zeros((TM, D), F32)

        x_copy(0).wait()

        def ln0_step(j, carry):
            words = _span(j, LN0_ROWS // 2)
            layernorm_to(words, xn_s.at[0, words, :])
            return carry
        lax.fori_loop(0, TM // LN0_ROWS, ln0_step, 0)

        def ffn_and_project(c, carry):
            m, part = c // KPARTS, c % KPARTS
            for cp in step_copies(c, True):
                cp.wait()
            acc_s[...] += ffn_step(_ld(xn_s[0]), *ffn_cols(c, True))
            permute_part(m, part)
            r = _dot(_ld(xn_s[0, :, _span(part, 2 * kw)]), _ld(wqkv_s[m, _span(part, kw), :]))
            for t in range(NT):
                qkv_s[m, t, HALO:HALO + TM, :] += r[:, t * 128:(t + 1) * 128]
            return carry
        lax.fori_loop(0, n_x, ffn_and_project, 0)

        wo_copy.start()
        x_copy(1).start()

        def start_x_tile(i, carry):
            x_copy(i).start()
            return carry
        lax.fori_loop(2, n_tiles, start_x_tile, 0)

        def ffn_and_attend(j, carry):
            c = n_x + j
            for cp in step_copies(c, False):
                cp.wait()
            acc_s[...] += ffn_step(_ld(xn_s[0]), *ffn_cols(c, False))
            for s in range(slabs_per_b):
                attention_slab(pl.multiple_of((j * slabs_per_b + s) * SLAB, SLAB), True)
            return carry
        lax.fori_loop(0, n_b, ffn_and_attend, 0)
        carry_halo()

        wo_copy.wait()
        x_copy(1).wait()

        def finish_tile0(j, carry):
            rows, words = _span(j, TAIL_ROWS), _span(j, TAIL_ROWS // 2)
            s = _dot(_ld(o_s[words, :]), _ld(wo_s[...]))
            res = _ld(x_s[words, :]).astype(F32) + s * _silu(acc_s[rows, :])
            out_s[words, :] = _pk(res.astype(BF16))
            layernorm_to(_span(j + TM // TAIL_ROWS, TAIL_ROWS // 2), xn_s.at[1, words, :])
            return carry
        lax.fori_loop(0, TM // TAIL_ROWS, finish_tile0, 0)
        out_copy(0).start()

        def tile_body(i, carry):
            slot = i & 1
            nxt = jnp.minimum(i + 1, n_tiles - 1)

            @pl.when(i + 1 < n_tiles)
            def _():
                x_copy(i + 1).wait()

            xn = _ld(xn_s[slot])
            for m in range(3):
                r = _dot(xn, _ld(wqkv_s[m]))
                for t in range(NT):
                    qkv_s[m, t, HALO:HALO + TM, :] = r[:, t * 128:(t + 1) * 128]

            layernorm_to(pl.ds(pl.multiple_of(nxt * hm, hm), hm), xn_s.at[1 - slot])

            acc = None
            done = 0
            for c in range(n_fc):
                d = ffn_step(_ld(xn_s[slot]), _span(c, FC), _span(c, FC // 2))
                acc = d if acc is None else acc + d
                for sl in range(done, SLABS_AFTER[c]):
                    attention_slab(sl * SLAB, False)
                done = SLABS_AFTER[c]
            carry_halo()

            s = _dot(_ld(o_s[...]), _ld(wo_s[...]))
            res = _ld(x_s[_span(i, hm), :]).astype(F32) + s * _silu(acc)
            out_s[_span(i, hm), :] = _pk(res.astype(BF16))
            out_copy(i).start()
            return carry

        lax.fori_loop(1, n_tiles, tile_body, 0)
        pltpu.make_async_copy(out_s, out_w, out_sem).wait()

    return kernel


def build(name="fused_block"):
    def fn(A_x, A_wqkv, A_wo, B_x, B_w_gate, B_w_up, B_w_down):
        del B_x
        B, S, D = A_x.shape
        F = B_w_gate.shape[1]
        assert B == 1 and D == NT * 128 and S % TM == 0 and S // TM >= 2 and F % FC == 0
        any_spec = pl.BlockSpec(memory_space=pl.ANY)
        out = pl.pallas_call(
            _make_kernel(S, D, F),
            in_specs=[any_spec] * 6,
            out_specs=any_spec,
            out_shape=jax.ShapeDtypeStruct((S, D), A_x.dtype),
            scratch_shapes=[
                pltpu.VMEM((S // 2, D), U32),
                pltpu.VMEM((S // 2, D), U32),
                pltpu.VMEM((3, D // 2, D), U32),
                pltpu.VMEM((D // 2, D), U32),
                pltpu.VMEM((D // 2, F), U32),
                pltpu.VMEM((D // 2, F), U32),
                pltpu.VMEM((F // 2, D), U32),
                pltpu.VMEM((2, TM // 2, D), U32),
                pltpu.VMEM((3, NT, HALO + TM, 128), F32),
                pltpu.VMEM((TM // 2, D), U32),
                pltpu.VMEM((TM, D), F32),
                pltpu.SemaphoreType.DMA((S // TM,)),
                pltpu.SemaphoreType.DMA(()),
                pltpu.SemaphoreType.DMA((3 * KPARTS + (F - 3 * KPARTS * PCX) // PCB + 1,)),
            ],
            compiler_params=pltpu.CompilerParams(vmem_limit_bytes=100 * 2 ** 20),
            name=name,
        )(A_x.reshape(S, D), A_wqkv, A_wo, B_w_gate, B_w_up, B_w_down)
        return out.reshape(B, S, D)
    return fn


_fused = build()


@jax.jit
def pallas_recurrent_scan__sliding_local_dilated__swiglu_ffn__prompt_kernel(
    A_x: jax.Array,
    A_wqkv: jax.Array,
    A_wo: jax.Array,
    B_x: jax.Array,
    B_w_gate: jax.Array,
    B_w_up: jax.Array,
    B_w_down: jax.Array,
):
    return _fused(A_x, A_wqkv, A_wo, B_x, B_w_gate, B_w_up, B_w_down)
```

```python
import functools

import jax
import jax.numpy as jnp
from jax import lax
import jax.experimental.pallas as pl
import jax.experimental.pallas.tpu as pltpu

H = 32
W = 8
DIL = 2
HALO = 16
NT = 8
EPS = 1e-5
LOG2E = 1.4426950408889634
MASKED = -1e9

TM = 256
FC = 512
PCX = 128
PCB = 256
KPARTS = 4
SLAB = 16
PERM_WORDS = 32
LN0_ROWS = 64
TAIL_ROWS = 128
SLABS_AFTER = (3, 6, 9, 12, 16, 16, 16)

F32 = jnp.float32
BF16 = jnp.bfloat16
U32 = jnp.uint32


def _dot(a, b):
    return jnp.dot(a, b, preferred_element_type=F32)


def _ld(words):
    return pltpu.bitcast(words, BF16)


def _pk(rows):
    return pltpu.bitcast(rows, U32)


def _silu(x):
    return x * pl.reciprocal(1.0 + jnp.exp(-x), approx=True)


def _span(i, n):
    return pl.ds(i * n, n) if isinstance(i, int) else pl.ds(pl.multiple_of(i * n, n), n)


def _group_bits(rows):
    lane = lax.broadcasted_iota(jnp.int32, (rows, 128), 1)
    return [((lane >> (2 + k)) & 1) == 1 for k in range(3)]


def _rotate_tiles(tiles, bits):
    x = [tiles[(-u) % NT] for u in range(NT)]
    for k in range(3):
        x = [jnp.where(bits[k], x[(t - (1 << k)) % NT], x[t]) for t in range(NT)]
    return x


def _permute_tiles(tiles, bits):
    x = [pltpu.roll(tiles[j], 4 * j, 1) if j else tiles[j] for j in range(NT)]
    x = _rotate_tiles(x, bits)
    return [pltpu.roll(x[t], 128 - 4 * t, 1) if t else x[t] for t in range(NT)]


def _unpermute_tiles(tiles, bits):
    x = [pltpu.roll(tiles[t], 4 * t, 1) if t else tiles[t] for t in range(NT)]
    x = _rotate_tiles(x, bits)
    return [pltpu.roll(x[j], 128 - 4 * j, 1) if j else x[j] for j in range(NT)]


def _make_kernel(S, D, F):
    n_tiles = S // TM
    n_fc = F // FC
    n_slabs = TM // SLAB
    hm = TM // 2
    kw = D // 2 // KPARTS
    n_x = 3 * KPARTS
    n_b = (F - n_x * PCX) // PCB
    slabs_per_b = n_slabs // n_b
    assert n_x * PCX + n_b * PCB == F
    assert n_b * slabs_per_b == n_slabs and len(SLABS_AFTER) == n_fc and SLABS_AFTER[-1] == n_slabs
    scale = (D // H) ** -0.5

    def kernel(x_hbm, wqkv_hbm, wo_hbm, wg_hbm, wu_hbm, wd_hbm, out_hbm,
               x_s, out_s, wqkv_s, wo_s, wg_s, wu_s, wd_s, xn_s, qkv_s, o_s, acc_s,
               x_sem, out_sem, w_sem):
        x_w, out_w = x_hbm.bitcast(U32), out_hbm.bitcast(U32)
        wqkv_w, wo_w = wqkv_hbm.bitcast(U32), wo_hbm.bitcast(U32)
        wg_w, wu_w, wd_w = wg_hbm.bitcast(U32), wu_hbm.bitcast(U32), wd_hbm.bitcast(U32)

        def x_copy(i):
            sem = w_sem.at[n_x + n_b] if isinstance(i, int) and i == 1 else x_sem.at[i]
            return pltpu.make_async_copy(x_w.at[_span(i, hm), :], x_s.at[_span(i, hm), :], sem)

        def out_copy(i):
            return pltpu.make_async_copy(out_s.at[_span(i, hm), :], out_w.at[_span(i, hm), :], out_sem)

        def ffn_cols(c, first_phase):
            if first_phase:
                return _span(c, PCX), _span(c, PCX // 2)
            start = n_x * PCX + (c - n_x) * PCB
            return pl.ds(pl.multiple_of(start, PCX), PCB), pl.ds(pl.multiple_of(start >> 1, PCX // 2), PCB // 2)

        def step_copies(c, first_phase):
            cols, drows = ffn_cols(c, first_phase)
            copies = [
                pltpu.make_async_copy(wg_w.at[:, cols], wg_s.at[:, cols], w_sem.at[c]),
                pltpu.make_async_copy(wu_w.at[:, cols], wu_s.at[:, cols], w_sem.at[c]),
            ]
            if first_phase:
                m, part = c // KPARTS, c % KPARTS
                copies.append(pltpu.make_async_copy(wqkv_w.at[_span(part, kw), _span(m, D)],
                                                    wqkv_s.at[m, _span(part, kw), :], w_sem.at[c]))
            copies.append(pltpu.make_async_copy(wd_w.at[drows, :], wd_s.at[drows, :], w_sem.at[c]))
            return copies

        wo_copy = pltpu.make_async_copy(wo_w, wo_s, w_sem.at[n_x + n_b])

        def layernorm_to(src_words, dst):
            words = x_s[src_words, :]
            halves = []
            for idx in range(2):
                x = pltpu.unpack_elementwise(words, index=idx, packed_dtype=BF16, unpacked_dtype=F32)
                mean = jnp.mean(x, axis=-1, keepdims=True)
                xc = x - mean
                var = jnp.mean(xc * xc, axis=-1, keepdims=True)
                halves.append(xc * lax.rsqrt(var + EPS))
            dst[...] = pltpu.pack_elementwise(halves, packed_dtype=BF16)

        def ffn_step(xn, cols, drows):
            g = _dot(xn, _ld(wg_s[:, cols]))
            u = _dot(xn, _ld(wu_s[:, cols]))
            h = (_silu(g) * u).astype(BF16)
            return _dot(h, _ld(wd_s[drows, :]))

        def permute_part(m, part):
            bits = _group_bits(PERM_WORDS)
            view = wqkv_s.at[m, _span(part, kw), :]
            for r in range(0, kw, PERM_WORDS):
                tiles = [view[r:r + PERM_WORDS, j * 128:(j + 1) * 128] for j in range(NT)]
                for t, val in enumerate(_permute_tiles(tiles, bits)):
                    view[r:r + PERM_WORDS, t * 128:(t + 1) * 128] = val

        def attention_slab(r0, first_tile):
            lane = lax.broadcasted_iota(jnp.int32, (SLAB, 128), 1)
            low1 = (lane & 1) == 0
            low2 = (lane & 2) == 0
            window = pl.ds(r0, HALO + SLAB)
            logit = [None] * W
            for t in range(NT):
                q = qkv_s[0, t, pl.ds(r0 + HALO, SLAB), :]
                k_win = qkv_s.at[1, t, window, :]
                for w in range(W):
                    off = HALO - DIL * w
                    prod = q * k_win[off:off + SLAB, :]
                    logit[w] = prod if logit[w] is None else logit[w] + prod
            if first_tile:
                row = lax.broadcasted_iota(jnp.int32, (SLAB, 128), 0) + r0
            for w in range(W):
                z = logit[w]
                z = z + jnp.where(low1, pltpu.roll(z, 127, 1), pltpu.roll(z, 1, 1))
                z = z + jnp.where(low2, pltpu.roll(z, 126, 1), pltpu.roll(z, 2, 1))
                if first_tile and w > 0:
                    z = jnp.where(row >= DIL * w, z, MASKED / scale)
                logit[w] = z
            top = functools.reduce(jnp.maximum, logit)
            e = [jnp.exp2((z - top) * (scale * LOG2E)) for z in logit]
            rinv = pl.reciprocal(functools.reduce(lambda a, b: a + b, e), approx=True)
            out = []
            for t in range(NT):
                v_win = qkv_s.at[2, t, window, :]
                acc = None
                for w in (0, 4, 1, 5, 2, 6, 3, 7):
                    off = HALO - DIL * w
                    prod = e[w] * v_win[off:off + SLAB, :]
                    acc = prod if acc is None else acc + prod
                out.append(_pk((acc * rinv).astype(BF16)))
            out = _unpermute_tiles(out, _group_bits(SLAB // 2))
            if isinstance(r0, int):
                words = pl.ds(r0 // 2, SLAB // 2)
            else:
                words = pl.ds(pl.multiple_of(r0 >> 1, SLAB // 2), SLAB // 2)
            for j in range(NT):
                o_s[words, j * 128:(j + 1) * 128] = out[j]

        def carry_halo():
            for m in (1, 2):
                for t in range(NT):
                    qkv_s[m, t, 0:HALO, :] = qkv_s[m, t, TM:TM + HALO, :]

        x_copy(0).start()

        def start_first_phase(c, carry):
            for cp in step_copies(c, True):
                cp.start()
            return carry
        lax.fori_loop(0, n_x, start_first_phase, 0)

        def start_second_phase(c, carry):
            for cp in step_copies(c, False):
                cp.start()
            return carry
        lax.fori_loop(n_x, n_x + n_b, start_second_phase, 0)

        for m in (1, 2):
            for t in range(NT):
                qkv_s[m, t, 0:HALO, :] = jnp.zeros((HALO, 128), F32)
        for m in range(3):
            for t in range(NT):
                qkv_s[m, t, HALO:HALO + TM, :] = jnp.zeros((TM, 128), F32)
        acc_s[...] = jnp.zeros((TM, D), F32)

        x_copy(0).wait()

        def ln0_step(j, carry):
            words = _span(j, LN0_ROWS // 2)
            layernorm_to(words, xn_s.at[0, words, :])
            return carry
        lax.fori_loop(0, TM // LN0_ROWS, ln0_step, 0)

        def ffn_and_project(c, carry):
            m, part = c // KPARTS, c % KPARTS
            for cp in step_copies(c, True):
                cp.wait()
            acc_s[...] += ffn_step(_ld(xn_s[0]), *ffn_cols(c, True))
            permute_part(m, part)
            r = _dot(_ld(xn_s[0, :, _span(part, 2 * kw)]), _ld(wqkv_s[m, _span(part, kw), :]))
            for t in range(NT):
                qkv_s[m, t, HALO:HALO + TM, :] += r[:, t * 128:(t + 1) * 128]
            return carry
        lax.fori_loop(0, n_x, ffn_and_project, 0)

        wo_copy.start()
        x_copy(1).start()

        def start_x_tile(i, carry):
            x_copy(i).start()
            return carry
        lax.fori_loop(2, n_tiles, start_x_tile, 0)

        def ffn_and_attend(j, carry):
            c = n_x + j
            for cp in step_copies(c, False):
                cp.wait()
            acc_s[...] += ffn_step(_ld(xn_s[0]), *ffn_cols(c, False))
            for s in range(slabs_per_b):
                attention_slab(pl.multiple_of((j * slabs_per_b + s) * SLAB, SLAB), True)
            return carry
        lax.fori_loop(0, n_b, ffn_and_attend, 0)
        carry_halo()

        wo_copy.wait()
        x_copy(1).wait()

        def finish_tile0(j, carry):
            rows, words = _span(j, TAIL_ROWS), _span(j, TAIL_ROWS // 2)
            s = _dot(_ld(o_s[words, :]), _ld(wo_s[...]))
            res = _ld(x_s[words, :]).astype(F32) + s * _silu(acc_s[rows, :])
            out_s[words, :] = _pk(res.astype(BF16))
            layernorm_to(_span(j + TM // TAIL_ROWS, TAIL_ROWS // 2), xn_s.at[1, words, :])
            return carry
        lax.fori_loop(0, TM // TAIL_ROWS, finish_tile0, 0)
        out_copy(0).start()

        def tile_body(i, carry):
            slot = i & 1
            nxt = jnp.minimum(i + 1, n_tiles - 1)

            @pl.when(i + 1 < n_tiles)
            def _():
                x_copy(i + 1).wait()

            xn = _ld(xn_s[slot])
            for m in range(3):
                r = _dot(xn, _ld(wqkv_s[m]))
                for t in range(NT):
                    qkv_s[m, t, HALO:HALO + TM, :] = r[:, t * 128:(t + 1) * 128]

            layernorm_to(pl.ds(pl.multiple_of(nxt * hm, hm), hm), xn_s.at[1 - slot])

            acc = None
            done = 0
            for c in range(n_fc):
                d = ffn_step(_ld(xn_s[slot]), _span(c, FC), _span(c, FC // 2))
                acc = d if acc is None else acc + d
                for sl in range(done, SLABS_AFTER[c]):
                    attention_slab(sl * SLAB, False)
                done = SLABS_AFTER[c]
            carry_halo()

            s = _dot(_ld(o_s[...]), _ld(wo_s[...]))
            res = _ld(x_s[_span(i, hm), :]).astype(F32) + s * _silu(acc)
            out_s[_span(i, hm), :] = _pk(res.astype(BF16))
            out_copy(i).start()
            return carry

        lax.fori_loop(1, n_tiles, tile_body, 0)
        pltpu.make_async_copy(out_s, out_w, out_sem).wait()

    return kernel


def build(name="fused_block"):
    def fn(A_x, A_wqkv, A_wo, B_x, B_w_gate, B_w_up, B_w_down):
        del B_x
        B, S, D = A_x.shape
        F = B_w_gate.shape[1]
        assert B == 1 and D == NT * 128 and S % TM == 0 and S // TM >= 2 and F % FC == 0
        any_spec = pl.BlockSpec(memory_space=pl.ANY)
        out = pl.pallas_call(
            _make_kernel(S, D, F),
            in_specs=[any_spec] * 6,
            out_specs=any_spec,
            out_shape=jax.ShapeDtypeStruct((S, D), A_x.dtype),
            scratch_shapes=[
                pltpu.VMEM((S // 2, D), U32),
                pltpu.VMEM((S // 2, D), U32),
                pltpu.VMEM((3, D // 2, D), U32),
                pltpu.VMEM((D // 2, D), U32),
                pltpu.VMEM((D // 2, F), U32),
                pltpu.VMEM((D // 2, F), U32),
                pltpu.VMEM((F // 2, D), U32),
                pltpu.VMEM((2, TM // 2, D), U32),
                pltpu.VMEM((3, NT, HALO + TM, 128), F32),
                pltpu.VMEM((TM // 2, D), U32),
                pltpu.VMEM((TM, D), F32),
                pltpu.SemaphoreType.DMA((S // TM,)),
                pltpu.SemaphoreType.DMA(()),
                pltpu.SemaphoreType.DMA((3 * KPARTS + (F - 3 * KPARTS * PCX) // PCB + 1,)),
            ],
            compiler_params=pltpu.CompilerParams(vmem_limit_bytes=100 * 2 ** 20),
            name=name,
        )(A_x.reshape(S, D), A_wqkv, A_wo, B_w_gate, B_w_up, B_w_down)
        return out.reshape(B, S, D)
    return fn


_fused = build()


@jax.jit
def pallas_recurrent_scan__sliding_local_dilated__swiglu_ffn__prompt_kernel(
    A_x: jax.Array,
    A_wqkv: jax.Array,
    A_wo: jax.Array,
    B_x: jax.Array,
    B_w_gate: jax.Array,
    B_w_up: jax.Array,
    B_w_down: jax.Array,
):
    return _fused(A_x, A_wqkv, A_wo, B_x, B_w_gate, B_w_up, B_w_down)
```

```python
import functools

import jax
import jax.numpy as jnp
from jax import lax
import jax.experimental.pallas as pl
import jax.experimental.pallas.tpu as pltpu

H = 32
W = 8
DIL = 2
HALO = 16
NT = 8
EPS = 1e-5
LOG2E = 1.4426950408889634
MASKED = -1e9

TM = 256
FC = 512
PCX = 128
PCB = 256
KPARTS = 4
SLAB = 16
PERM_WORDS = 32
LN0_ROWS = 64
TAIL_ROWS = 128
SLABS_AFTER = (2, 5, 8, 11, 14, 16, 16)

F32 = jnp.float32
BF16 = jnp.bfloat16
U32 = jnp.uint32


def _dot(a, b):
    return jnp.dot(a, b, preferred_element_type=F32)


def _ld(words):
    return pltpu.bitcast(words, BF16)


def _pk(rows):
    return pltpu.bitcast(rows, U32)


def _silu(x):
    return x * pl.reciprocal(1.0 + jnp.exp(-x), approx=True)


def _span(i, n):
    return pl.ds(i * n, n) if isinstance(i, int) else pl.ds(pl.multiple_of(i * n, n), n)


def _group_bits(rows):
    lane = lax.broadcasted_iota(jnp.int32, (rows, 128), 1)
    return [((lane >> (2 + k)) & 1) == 1 for k in range(3)]


def _rotate_tiles(tiles, bits):
    x = [tiles[(-u) % NT] for u in range(NT)]
    for k in range(3):
        x = [jnp.where(bits[k], x[(t - (1 << k)) % NT], x[t]) for t in range(NT)]
    return x


def _permute_tiles(tiles, bits):
    x = [pltpu.roll(tiles[j], 4 * j, 1) if j else tiles[j] for j in range(NT)]
    x = _rotate_tiles(x, bits)
    return [pltpu.roll(x[t], 128 - 4 * t, 1) if t else x[t] for t in range(NT)]


def _unpermute_tiles(tiles, bits):
    x = [pltpu.roll(tiles[t], 4 * t, 1) if t else tiles[t] for t in range(NT)]
    x = _rotate_tiles(x, bits)
    return [pltpu.roll(x[j], 128 - 4 * j, 1) if j else x[j] for j in range(NT)]


def _make_kernel(S, D, F):
    n_tiles = S // TM
    n_fc = F // FC
    n_slabs = TM // SLAB
    hm = TM // 2
    kw = D // 2 // KPARTS
    n_x = 3 * KPARTS
    n_b = (F - n_x * PCX) // PCB
    slabs_per_b = n_slabs // n_b
    assert n_x * PCX + n_b * PCB == F
    assert n_b * slabs_per_b == n_slabs and len(SLABS_AFTER) == n_fc and SLABS_AFTER[-1] == n_slabs
    scale = (D // H) ** -0.5

    def kernel(x_hbm, wqkv_hbm, wo_hbm, wg_hbm, wu_hbm, wd_hbm, out_hbm,
               x_s, out_s, wqkv_s, wo_s, wg_s, wu_s, wd_s, xn_s, qkv_s, o_s, acc_s,
               x_sem, out_sem, w_sem, *qo_s):
        x_w, out_w = x_hbm.bitcast(U32), out_hbm.bitcast(U32)
        wqkv_w, wo_w = wqkv_hbm.bitcast(U32), wo_hbm.bitcast(U32)
        wg_w, wu_w, wd_w = wg_hbm.bitcast(U32), wu_hbm.bitcast(U32), wd_hbm.bitcast(U32)

        def x_copy(i):
            sem = w_sem.at[n_x + n_b] if isinstance(i, int) and i == 1 else x_sem.at[i]
            return pltpu.make_async_copy(x_w.at[_span(i, hm), :], x_s.at[_span(i, hm), :], sem)

        def out_copy(i):
            return pltpu.make_async_copy(out_s.at[_span(i, hm), :], out_w.at[_span(i, hm), :], out_sem)

        def ffn_cols(c, first_phase):
            if first_phase:
                return _span(c, PCX), _span(c, PCX // 2)
            start = n_x * PCX + (c - n_x) * PCB
            return pl.ds(pl.multiple_of(start, PCX), PCB), pl.ds(pl.multiple_of(start >> 1, PCX // 2), PCB // 2)

        def step_copies(c, first_phase):
            cols, drows = ffn_cols(c, first_phase)
            copies = [
                pltpu.make_async_copy(wg_w.at[:, cols], wg_s.at[:, cols], w_sem.at[c]),
                pltpu.make_async_copy(wu_w.at[:, cols], wu_s.at[:, cols], w_sem.at[c]),
            ]
            if first_phase:
                m, part = c // KPARTS, c % KPARTS
                copies.append(pltpu.make_async_copy(wqkv_w.at[_span(part, kw), _span(m, D)],
                                                    wqkv_s.at[m, _span(part, kw), :], w_sem.at[c]))
            copies.append(pltpu.make_async_copy(wd_w.at[drows, :], wd_s.at[drows, :], w_sem.at[c]))
            return copies

        wo_copy = pltpu.make_async_copy(wo_w, wo_s, w_sem.at[n_x + n_b])

        def layernorm_to(src_words, dst):
            words = x_s[src_words, :]
            halves = []
            for idx in range(2):
                x = pltpu.unpack_elementwise(words, index=idx, packed_dtype=BF16, unpacked_dtype=F32)
                mean = jnp.mean(x, axis=-1, keepdims=True)
                xc = x - mean
                var = jnp.mean(xc * xc, axis=-1, keepdims=True)
                halves.append(xc * lax.rsqrt(var + EPS))
            dst[...] = pltpu.pack_elementwise(halves, packed_dtype=BF16)

        def ffn_step(xn, cols, drows):
            g = _dot(xn, _ld(wg_s[:, cols]))
            u = _dot(xn, _ld(wu_s[:, cols]))
            h = (_silu(g) * u).astype(BF16)
            return _dot(h, _ld(wd_s[drows, :]))

        def permute_part(m, part):
            bits = _group_bits(PERM_WORDS)
            view = wqkv_s.at[m, _span(part, kw), :]
            for r in range(0, kw, PERM_WORDS):
                tiles = [view[r:r + PERM_WORDS, j * 128:(j + 1) * 128] for j in range(NT)]
                for t, val in enumerate(_permute_tiles(tiles, bits)):
                    view[r:r + PERM_WORDS, t * 128:(t + 1) * 128] = val

        def attention_slab(r0, q_tile, put_o, first_tile):
            lane = lax.broadcasted_iota(jnp.int32, (SLAB, 128), 1)
            low1 = (lane & 1) == 0
            low2 = (lane & 2) == 0
            window = pl.ds(r0, HALO + SLAB)
            logit = [None] * W
            for t in range(NT):
                q = q_tile(t)
                k_win = qkv_s.at[1, t, window, :]
                for w in range(W):
                    off = HALO - DIL * w
                    prod = q * k_win[off:off + SLAB, :]
                    logit[w] = prod if logit[w] is None else logit[w] + prod
            if first_tile:
                row = lax.broadcasted_iota(jnp.int32, (SLAB, 128), 0) + r0
            for w in range(W):
                z = logit[w]
                z = z + jnp.where(low1, pltpu.roll(z, 127, 1), pltpu.roll(z, 1, 1))
                z = z + jnp.where(low2, pltpu.roll(z, 126, 1), pltpu.roll(z, 2, 1))
                if first_tile and w > 0:
                    z = jnp.where(row >= DIL * w, z, MASKED / scale)
                logit[w] = z
            top = functools.reduce(jnp.maximum, logit)
            e = [jnp.exp2((z - top) * (scale * LOG2E)) for z in logit]
            rinv = pl.reciprocal(functools.reduce(lambda a, b: a + b, e), approx=True)
            out = []
            for t in range(NT):
                v_win = qkv_s.at[2, t, window, :]
                acc = None
                for w in (0, 4, 1, 5, 2, 6, 3, 7):
                    off = HALO - DIL * w
                    prod = e[w] * v_win[off:off + SLAB, :]
                    acc = prod if acc is None else acc + prod
                out.append(_pk((acc * rinv).astype(BF16)))
            out = _unpermute_tiles(out, _group_bits(SLAB // 2))
            for j in range(NT):
                put_o(j, out[j])

        def carry_halo():
            for m in (1, 2):
                for t in range(NT):
                    qkv_s[m, t, 0:HALO, :] = qkv_s[m, t, TM:TM + HALO, :]

        x_copy(0).start()

        def start_first_phase(c, carry):
            for cp in step_copies(c, True):
                cp.start()
            return carry
        lax.fori_loop(0, n_x, start_first_phase, 0)

        def start_second_phase(c, carry):
            for cp in step_copies(c, False):
                cp.start()
            return carry
        lax.fori_loop(n_x, n_x + n_b, start_second_phase, 0)

        for m in (1, 2):
            for t in range(NT):
                qkv_s[m, t, 0:HALO, :] = jnp.zeros((HALO, 128), F32)
        for m in range(3):
            for t in range(NT):
                qkv_s[m, t, HALO:HALO + TM, :] = jnp.zeros((TM, 128), F32)
        acc_s[...] = jnp.zeros((TM, D), F32)

        x_copy(0).wait()

        def ln0_step(j, carry):
            words = _span(j, LN0_ROWS // 2)
            layernorm_to(words, xn_s.at[0, words, :])
            return carry
        lax.fori_loop(0, TM // LN0_ROWS, ln0_step, 0)

        def ffn_and_project(c, carry):
            m, part = c // KPARTS, c % KPARTS
            for cp in step_copies(c, True):
                cp.wait()
            acc_s[...] += ffn_step(_ld(xn_s[0]), *ffn_cols(c, True))
            permute_part(m, part)
            r = _dot(_ld(xn_s[0, :, _span(part, 2 * kw)]), _ld(wqkv_s[m, _span(part, kw), :]))
            for t in range(NT):
                qkv_s[m, t, HALO:HALO + TM, :] += r[:, t * 128:(t + 1) * 128]
            return carry
        lax.fori_loop(0, n_x, ffn_and_project, 0)

        wo_copy.start()
        x_copy(1).start()

        def start_x_tile(i, carry):
            x_copy(i).start()
            return carry
        lax.fori_loop(2, n_tiles, start_x_tile, 0)

        def ffn_and_attend(j, carry):
            c = n_x + j
            for cp in step_copies(c, False):
                cp.wait()
            acc_s[...] += ffn_step(_ld(xn_s[0]), *ffn_cols(c, False))
            for s in range(slabs_per_b):
                r0 = pl.multiple_of((j * slabs_per_b + s) * SLAB, SLAB)
                words = pl.ds(pl.multiple_of(r0 >> 1, SLAB // 2), SLAB // 2)

                def put_o(t, val, words=words):
                    o_s[words, t * 128:(t + 1) * 128] = val

                attention_slab(r0, lambda t, r0=r0: qkv_s[0, t, pl.ds(r0 + HALO, SLAB), :], put_o, True)
            return carry
        lax.fori_loop(0, n_b, ffn_and_attend, 0)
        carry_halo()

        wo_copy.wait()
        x_copy(1).wait()

        def finish_tile0(j, carry):
            rows, words = _span(j, TAIL_ROWS), _span(j, TAIL_ROWS // 2)
            s = _dot(_ld(o_s[words, :]), _ld(wo_s[...]))
            res = _ld(x_s[words, :]).astype(F32) + s * _silu(acc_s[rows, :])
            out_s[words, :] = _pk(res.astype(BF16))
            layernorm_to(_span(j + TM // TAIL_ROWS, TAIL_ROWS // 2), xn_s.at[1, words, :])
            return carry
        lax.fori_loop(0, TM // TAIL_ROWS, finish_tile0, 0)
        out_copy(0).start()

        def tile_body(i, carry):
            slot = i & 1
            nxt = jnp.minimum(i + 1, n_tiles - 1)

            @pl.when(i + 1 < n_tiles)
            def _():
                x_copy(i + 1).wait()

            q_slot = jnp.minimum(i, 1)
            o_slot = jnp.minimum(i + 1, 2)

            xn = _ld(xn_s[slot])
            for m in range(3):
                r = _dot(xn, _ld(wqkv_s[m]))
                if m == 0:
                    for sl in range(n_slabs):
                        qo_s[sl][q_slot] = r[sl * SLAB:(sl + 1) * SLAB, :]
                else:
                    for t in range(NT):
                        qkv_s[m, t, HALO:HALO + TM, :] = r[:, t * 128:(t + 1) * 128]

            layernorm_to(pl.ds(pl.multiple_of(nxt * hm, hm), hm), xn_s.at[1 - slot])

            acc = None
            done = 0
            for c in range(n_fc):
                d = ffn_step(_ld(xn_s[slot]), _span(c, FC), _span(c, FC // 2))
                acc = d if acc is None else acc + d
                for sl in range(done, SLABS_AFTER[c]):
                    def put_o(t, val, sl=sl):
                        qo_s[sl][o_slot, 0:SLAB // 2, t * 128:(t + 1) * 128] = pltpu.bitcast(val, F32)

                    attention_slab(sl * SLAB, lambda t, sl=sl: qo_s[sl][q_slot, :, t * 128:(t + 1) * 128],
                                   put_o, False)
                done = SLABS_AFTER[c]
            carry_halo()

            o = jnp.concatenate([pltpu.bitcast(buf[o_slot, 0:SLAB // 2, :], BF16) for buf in qo_s], axis=0)
            s = _dot(o, _ld(wo_s[...]))
            res = _ld(x_s[_span(i, hm), :]).astype(F32) + s * _silu(acc)
            out_s[_span(i, hm), :] = _pk(res.astype(BF16))
            out_copy(i).start()
            return carry

        lax.fori_loop(1, n_tiles, tile_body, 0)
        pltpu.make_async_copy(out_s, out_w, out_sem).wait()

    return kernel


def build(name="fused_block"):
    def fn(A_x, A_wqkv, A_wo, B_x, B_w_gate, B_w_up, B_w_down):
        del B_x
        B, S, D = A_x.shape
        F = B_w_gate.shape[1]
        assert B == 1 and D == NT * 128 and S % TM == 0 and S // TM >= 2 and F % FC == 0
        any_spec = pl.BlockSpec(memory_space=pl.ANY)
        out = pl.pallas_call(
            _make_kernel(S, D, F),
            in_specs=[any_spec] * 6,
            out_specs=any_spec,
            out_shape=jax.ShapeDtypeStruct((S, D), A_x.dtype),
            scratch_shapes=[
                pltpu.VMEM((S // 2, D), U32),
                pltpu.VMEM((S // 2, D), U32),
                pltpu.VMEM((3, D // 2, D), U32),
                pltpu.VMEM((D // 2, D), U32),
                pltpu.VMEM((D // 2, F), U32),
                pltpu.VMEM((D // 2, F), U32),
                pltpu.VMEM((F // 2, D), U32),
                pltpu.VMEM((2, TM // 2, D), U32),
                pltpu.VMEM((3, NT, HALO + TM, 128), F32),
                pltpu.VMEM((TM // 2, D), U32),
                pltpu.VMEM((TM, D), F32),
                pltpu.SemaphoreType.DMA((S // TM,)),
                pltpu.SemaphoreType.DMA(()),
                pltpu.SemaphoreType.DMA((3 * KPARTS + (F - 3 * KPARTS * PCX) // PCB + 1,)),
            ] + [pltpu.VMEM((3, SLAB, D), F32)] * (TM // SLAB),
            compiler_params=pltpu.CompilerParams(vmem_limit_bytes=100 * 2 ** 20),
            name=name,
        )(A_x.reshape(S, D), A_wqkv, A_wo, B_w_gate, B_w_up, B_w_down)
        return out.reshape(B, S, D)
    return fn


_fused = build()


@jax.jit
def pallas_recurrent_scan__sliding_local_dilated__swiglu_ffn__prompt_kernel(
    A_x: jax.Array,
    A_wqkv: jax.Array,
    A_wo: jax.Array,
    B_x: jax.Array,
    B_w_gate: jax.Array,
    B_w_up: jax.Array,
    B_w_down: jax.Array,
):
    return _fused(A_x, A_wqkv, A_wo, B_x, B_w_gate, B_w_up, B_w_down)
```
